```python
import os as _os
_os.environ.setdefault("JAX_PLATFORMS", "cpu")
import jax
import jax.numpy as jnp

def _softmax(x, axis=-1):
    return jax.nn.softmax(x, axis=axis)
def _gelu(x):
    return jax.nn.gelu(x, approximate=True)
def _silu(x):
    return jax.nn.silu(x)
def _sigmoid(x):
    return jax.nn.sigmoid(x)
def _layernorm(x, axis=-1, eps=1e-5):
    m = jnp.mean(x, axis=axis, keepdims=True)
    v = jnp.var(x, axis=axis, keepdims=True)
    return (x - m) / jnp.sqrt(v + eps)
def _scatter_add(tgt, idx, src, axis=0):
    return tgt.at[idx].add(src)
def _segment_sum(src, seg, n):
    return jax.ops.segment_sum(src, seg, n)
class _Rng:
    def __init__(self, key):
        self._k = key
    def _next(self):
        self._k, sub = jax.random.split(self._k)
        return sub
    def normal(self, shape):
        return jax.random.normal(self._next(), shape, dtype=jnp.bfloat16)
    def randint(self, lo, hi, shape):
        return jax.random.randint(self._next(), shape, lo, hi, dtype=jnp.int32)
    def uniform(self, shape, lo=0.0, hi=1.0):
        return jax.random.uniform(self._next(), shape, jnp.bfloat16, lo, hi)
    def permutation(self, n):
        return jax.random.permutation(self._next(), n)


kernel_name = 'gated_mix__ssm_conv_s5__geglu_ffn__prompt'

def setup_inputs():
    _rng = _Rng(jax.random.key(int.from_bytes(__import__("os").urandom(4), "little")))
    _w = (lambda a: (lambda t: t.astype(jnp.bfloat16) if jnp.issubdtype(t.dtype, jnp.floating) else t)(jnp.asarray(a)))
    def _A_setup():
        B, S, D = 1, 2048, 512
        P = D
        Lambda_re = -0.5 * jnp.exp((lambda *s: _rng.normal(s) * 0.4)(P))
        Lambda_im = (lambda *s: _rng.normal(s) * 0.4)(P) * 1.0
        B_re = (lambda *s: _rng.normal(s) * 0.4)(P, D) * (D ** -0.5)
        B_im = (lambda *s: _rng.normal(s) * 0.4)(P, D) * (D ** -0.5)
        C_re = (lambda *s: _rng.normal(s) * 0.4)(D, P) * (P ** -0.5)
        C_im = (lambda *s: _rng.normal(s) * 0.4)(D, P) * (P ** -0.5)
        log_dt = (lambda *s: _rng.normal(s) * 0.4)(P) * 0.3 - 2.0
        Dskip = (lambda *s: _rng.normal(s) * 0.4)(D)
        return {
            "x": _w((lambda *s: _rng.normal(s) * 0.05)(B, S, D)),
            "Lambda_re": _w(Lambda_re),
            "Lambda_im": _w(Lambda_im),
            "B_re": _w(B_re),
            "B_im": _w(B_im),
            "C_re": _w(C_re),
            "C_im": _w(C_im),
            "log_dt": _w(log_dt),
            "Dskip": _w(Dskip),
        }
    _A_in = _A_setup()

    def _B_setup():
        B, S, D, F = 1, 2048, 512, 1376
        return {
            "x": _w((lambda *s: _rng.normal(s) * 0.05)(B, S, D)),
            "w_gate": _w((lambda *s: _rng.normal(s) * 0.1)(D, F)),
            "w_up": _w((lambda *s: _rng.normal(s) * 0.1)(D, F)),
            "w_down": _w((lambda *s: _rng.normal(s) * 0.1)(F, D)),
        }
    _B_in = _B_setup()

    return {
        "A_x": _A_in["x"],
        "A_Lambda_re": _A_in["Lambda_re"],
        "A_Lambda_im": _A_in["Lambda_im"],
        "A_B_re": _A_in["B_re"],
        "A_B_im": _A_in["B_im"],
        "A_C_re": _A_in["C_re"],
        "A_C_im": _A_in["C_im"],
        "A_log_dt": _A_in["log_dt"],
        "A_Dskip": _A_in["Dskip"],
        "B_x": _B_in["x"],
        "B_w_gate": _B_in["w_gate"],
        "B_w_up": _B_in["w_up"],
        "B_w_down": _B_in["w_down"],
        "gate_w": _w((lambda *s: _rng.normal(s) * 0.05)(512) * 16.0),
    }

def reference(A_x, A_Lambda_re, A_Lambda_im, A_B_re, A_B_im, A_C_re, A_C_im, A_log_dt, A_Dskip, B_x, B_w_gate, B_w_up, B_w_down, gate_w):
    def _A_ref(x, Lambda_re, Lambda_im, B_re, B_im, C_re, C_im, log_dt, Dskip):
        Bsz, L, H = x.shape
        Lam = Lambda_re + 1j * Lambda_im
        Bmat = B_re + 1j * B_im
        Cmat = C_re + 1j * C_im
        dt = jnp.exp(log_dt)
        Lam_bar = jnp.exp(dt * Lam)
        B_bar = ((Lam_bar - 1.0) / Lam)[:, None] * Bmat
        Bu = jnp.einsum("bld,pd->blp", x + 0j, B_bar)
        h = jnp.zeros_like(Bu[:, 0, :])
        hs = []
        for t in range(L):
            h = Lam_bar[None, :] * h + Bu[:, t, :]
            hs.append(h)
        hseq = jnp.stack(hs, 1)
        y = 2.0 * jnp.einsum("blp,dp->bld", hseq, Cmat).real + x * Dskip[None, None, :]
        return y

    def _B_ref(x, w_gate, w_up, w_down):
        return (_gelu(x @ w_gate) * (x @ w_up)) @ w_down

    x = A_x
    g = _sigmoid((x * gate_w).sum(-1, keepdims=True))
    a = _A_ref(x, A_Lambda_re, A_Lambda_im, A_B_re, A_B_im, A_C_re, A_C_im, A_log_dt, A_Dskip)
    b = _B_ref(x, B_w_gate, B_w_up, B_w_down)
    return g * a + (1 - g) * b
```

```python
import jax
import jax.numpy as jnp
import jax.experimental.pallas as pl
import jax.experimental.pallas.tpu as pltpu

_T = 256
_NSEG = 8
_SEG = _T // _NSEG
_FT = 128

_NT = (((1,), (1,)), ((), ()))


def _gelu_tanh(v):
    c = 0.7978845608028654
    return 0.5 * v * (1.0 + jnp.tanh(c * (v + 0.044715 * (v * v * v))))


def _kernel(x_ref, lre_ref, lim_ref, ldt_ref, bre_ref, bim_ref,
            cre_hbm, cim_hbm, dskip_ref, wg_hbm, wu_hbm, wd_hbm, gw_ref,
            o_ref,
            bcat_ref, ccat_ref, apow_ref, carry_ref, perm_ref, h_ref, bu_ref, yp_ref, hid_ref,
            wg_ref, wu_ref, wd_ref, sems):
    P = bre_ref.shape[0]
    F = wd_ref.shape[0]
    D = x_ref.shape[1]
    step = pl.program_id(0)
    f32 = jnp.float32
    row = lambda r: r[...].astype(f32).reshape(1, r.shape[0])

    copies = [
        pltpu.make_async_copy(wg_hbm, wg_ref, sems.at[0]),
        pltpu.make_async_copy(wu_hbm, wu_ref, sems.at[1]),
        pltpu.make_async_copy(cre_hbm, ccat_ref.at[0], sems.at[2]),
        pltpu.make_async_copy(cim_hbm, ccat_ref.at[1], sems.at[3]),
        pltpu.make_async_copy(wd_hbm, wd_ref, sems.at[4]),
    ]

    @pl.when(step == 0)
    def _init():
        for c in copies:
            c.start()
        dt = jnp.exp(row(ldt_ref)).astype(jnp.bfloat16).astype(f32)
        lr = row(lre_ref)
        li = row(lim_ref)
        mag = jnp.exp(dt * lr)
        ar = mag * jnp.cos(dt * li)
        ai = mag * jnp.sin(dt * li)
        nr = ar - 1.0
        den = lr * lr + li * li
        cr = (nr * lr + ai * li) / den
        ci = (ai * lr - nr * li) / den
        rows = jax.lax.broadcasted_iota(jnp.int32, (8, P), 0)
        cct = jnp.where(rows == 0, cr, ci).T
        cr_c = cct[:, 0:1]
        ci_c = cct[:, 1:2]
        bre = bre_ref[...].astype(f32)
        bim = bim_ref[...].astype(f32)
        bcat_ref[0:P, :] = (cr_c * bre - ci_c * bim).astype(jnp.bfloat16)
        bcat_ref[P:2 * P, :] = (cr_c * bim + ci_c * bre).astype(jnp.bfloat16)
        pr, pi = ar, ai
        for k in range(_SEG):
            apow_ref[k:k + 1, 0:P] = pr
            apow_ref[k:k + 1, P:2 * P] = pi
            pr, pi = pr * ar - pi * ai, pr * ai + pi * ar
        carry_ref[...] = jnp.zeros(carry_ref.shape, f32)
        rp = jax.lax.broadcasted_iota(jnp.int32, (_T, _T), 0)
        cn = jax.lax.broadcasted_iota(jnp.int32, (_T, _T), 1)
        src = (rp % _NSEG) * _SEG + rp // _NSEG
        perm_ref[...] = jnp.where(cn == src, 1.0, 0.0).astype(jnp.bfloat16)

    def body(first):
        def wait_first(*idx):
            if first:
                for i in idx:
                    copies[i].wait()

        x = x_ref[...]

        xp = jnp.dot(perm_ref[...], x, preferred_element_type=f32).astype(jnp.bfloat16)
        bu_ref[...] = jax.lax.dot_general(xp, bcat_ref[...], _NT, preferred_element_type=f32)

        def scan_steps():
            a_re = jnp.broadcast_to(apow_ref[0:1, 0:P], (_NSEG, P))
            a_im = jnp.broadcast_to(apow_ref[0:1, P:2 * P], (_NSEG, P))
            c_re = carry_ref[:, 0:P]
            c_im = carry_ref[:, P:2 * P]
            h_re, h_im = c_re, c_im
            for i in range(_SEG):
                b_re = bu_ref[i * _NSEG:(i + 1) * _NSEG, 0:P]
                b_im = bu_ref[i * _NSEG:(i + 1) * _NSEG, P:2 * P]
                h_re, h_im = (a_re * h_re - a_im * h_im + b_re,
                              a_re * h_im + a_im * h_re + b_im)
                yield
            aS_re = apow_ref[_SEG - 1:_SEG, 0:P]
            aS_im = apow_ref[_SEG - 1:_SEG, P:2 * P]
            e_re = h_re[0:1]
            e_im = h_im[0:1]
            rows_re = [c_re[0:1]]
            rows_im = [c_im[0:1]]
            for j in range(1, _NSEG):
                rows_re.append(e_re)
                rows_im.append(e_im)
                e_re, e_im = (h_re[j:j + 1] + aS_re * e_re - aS_im * e_im,
                              h_im[j:j + 1] + aS_re * e_im + aS_im * e_re)
            h_re = jnp.concatenate(rows_re, axis=0)
            h_im = jnp.concatenate(rows_im, axis=0)
            row0 = jax.lax.broadcasted_iota(jnp.int32, (_NSEG, P), 0) == 0
            carry_ref[:, 0:P] = jnp.where(row0, jnp.broadcast_to(e_re, (_NSEG, P)), 0.0)
            carry_ref[:, P:2 * P] = jnp.where(row0, jnp.broadcast_to(e_im, (_NSEG, P)), 0.0)
            yield
            for i in range(_SEG):
                b_re = bu_ref[i * _NSEG:(i + 1) * _NSEG, 0:P]
                b_im = bu_ref[i * _NSEG:(i + 1) * _NSEG, P:2 * P]
                h_re, h_im = (a_re * h_re - a_im * h_im + b_re,
                              a_re * h_im + a_im * h_re + b_im)
                if i % 2 == 0:
                    prev = (h_re, h_im)
                else:
                    r0 = (i - 1) * _NSEG
                    h_ref[r0:r0 + 2 * _NSEG, 0:P] = jnp.concatenate(
                        [prev[0], h_re], axis=0).astype(jnp.bfloat16)
                    h_ref[r0:r0 + 2 * _NSEG, P:2 * P] = jnp.concatenate(
                        [prev[1], h_im], axis=0).astype(jnp.bfloat16)
                yield

        scan = scan_steps()
        n_scan = 2 * _SEG + 1

        wait_first(0, 1)
        tiles = [(f0, min(_FT, F - f0)) for f0 in range(0, F, _FT)]
        done = 0
        for k, (f0, fw) in enumerate(tiles):
            gate = jax.lax.dot_general(x, wg_ref[f0:f0 + fw, :], _NT,
                                       preferred_element_type=f32)
            up = jax.lax.dot_general(x, wu_ref[f0:f0 + fw, :], _NT,
                                     preferred_element_type=f32)
            hid_ref[:, f0:f0 + fw] = (_gelu_tanh(gate) * up).astype(jnp.bfloat16)
            target = (n_scan * (k + 1)) // len(tiles)
            while done < target:
                next(scan)
                done += 1

        wait_first(2, 3)
        h_re = h_ref[:, 0:P]
        h_im = h_ref[:, P:2 * P]
        yp = (jax.lax.dot_general(h_re, ccat_ref[0], _NT, preferred_element_type=f32)
              - jax.lax.dot_general(h_im, ccat_ref[1], _NT, preferred_element_type=f32))
        for g in range(D // 128):
            yp_ref[g] = yp[:, g * 128:(g + 1) * 128]
        tiles_y = []
        for m in range(_T // 8):
            j, i0 = (8 * m) // _SEG, (8 * m) % _SEG
            tiles_y.append(jnp.concatenate(
                [yp_ref[g, pl.ds(i0 * _NSEG + j, 8, stride=_NSEG), :] for g in range(D // 128)],
                axis=1))
        y = jnp.concatenate(tiles_y, axis=0)
        xf = x.astype(f32)
        a_out = 2.0 * y + xf * row(dskip_ref)

        wait_first(4)
        b_out = jnp.dot(hid_ref[...], wd_ref[...], preferred_element_type=f32)

        s = jnp.sum(xf * row(gw_ref), axis=-1, keepdims=True)
        g = 1.0 / (1.0 + jnp.exp(-s))
        o_ref[...] = g * a_out + (1.0 - g) * b_out

    pl.when(step == 0)(lambda: body(True))
    pl.when(step != 0)(lambda: body(False))


@jax.jit
def pallas_gated_mix__ssm_conv_s5__geglu_ffn__prompt_kernel(
    A_x: jax.Array,
    A_Lambda_re: jax.Array,
    A_Lambda_im: jax.Array,
    A_B_re: jax.Array,
    A_B_im: jax.Array,
    A_C_re: jax.Array,
    A_C_im: jax.Array,
    A_log_dt: jax.Array,
    A_Dskip: jax.Array,
    B_x: jax.Array,
    B_w_gate: jax.Array,
    B_w_up: jax.Array,
    B_w_down: jax.Array,
    gate_w: jax.Array,
):
    Bsz, L, D = A_x.shape
    P = A_B_re.shape[0]
    F = B_w_gate.shape[1]
    assert Bsz == 1 and L % _T == 0
    x2 = A_x.reshape(L, D)

    full = lambda shape: pl.BlockSpec(shape, lambda i: (0,) * len(shape))
    hbm = pl.BlockSpec(memory_space=pl.ANY)

    out = pl.pallas_call(
        _kernel,
        grid=(L // _T,),
        in_specs=[
            pl.BlockSpec((_T, D), lambda i: (i, 0)),
            full((P,)), full((P,)), full((P,)),
            full((P, D)), full((P, D)),
            hbm, hbm,
            full((D,)),
            hbm, hbm, hbm,
            full((D,)),
        ],
        out_specs=pl.BlockSpec((_T, D), lambda i: (i, 0)),
        out_shape=jax.ShapeDtypeStruct((L, D), jnp.float32),
        scratch_shapes=[
            pltpu.VMEM((2 * P, D), jnp.bfloat16),
            pltpu.VMEM((2, D, P), jnp.bfloat16),
            pltpu.VMEM((_SEG, 2 * P), jnp.float32),
            pltpu.VMEM((_NSEG, 2 * P), jnp.float32),
            pltpu.VMEM((_T, _T), jnp.bfloat16),
            pltpu.VMEM((_T, 2 * P), jnp.bfloat16),
            pltpu.VMEM((_T, 2 * P), jnp.float32),
            pltpu.VMEM((D // 128, _T, 128), jnp.float32),
            pltpu.VMEM((_T, F), jnp.bfloat16),
            pltpu.VMEM((F, D), jnp.bfloat16),
            pltpu.VMEM((F, D), jnp.bfloat16),
            pltpu.VMEM((F, D), jnp.bfloat16),
            pltpu.SemaphoreType.DMA((5,)),
        ],
        compiler_params=pltpu.CompilerParams(
            dimension_semantics=("arbitrary",),
            vmem_limit_bytes=100 * 1024 * 1024,
        ),
    )(x2, A_Lambda_re, A_Lambda_im, A_log_dt,
      A_B_re, A_B_im, A_C_re, A_C_im, A_Dskip,
      B_w_gate.T, B_w_up.T, B_w_down, gate_w)
    return out.reshape(Bsz, L, D)
```

```python
import jax
import jax.numpy as jnp
import jax.experimental.pallas as pl
import jax.experimental.pallas.tpu as pltpu

_T = 256
_FT = 128
_DG = 4

_NT = (((1,), (1,)), ((), ()))


def _gelu_tanh(v):
    c = 0.7978845608028654
    return 0.5 * v * (1.0 + jnp.tanh(c * (v + 0.044715 * (v * v * v))))


def _kernel(x_ref, lre_ref, lim_ref, ldt_ref, bre_hbm, bim_hbm,
            cre_hbm, cim_hbm, dskip_ref, wg_hbm, wu_hbm, wd_hbm, gw_ref,
            o_ref,
            braw_ref, bcat_ref, ccat_ref, tab_ref, carry_ref, h_ref, bu_ref,
            hid_ref, wg_ref, wu_ref, wd_ref, sems):
    P = bre_hbm.shape[0]
    F = wd_ref.shape[0]
    step = pl.program_id(0)
    f32 = jnp.float32
    bf16 = jnp.bfloat16
    row = lambda r: r[...].astype(f32).reshape(1, r.shape[0])
    tiles = [(f0, min(_FT, F - f0)) for f0 in range(0, F, _FT)]

    copies = {}

    def add_copy(name, src, dst):
        copies[name] = pltpu.make_async_copy(src, dst, sems.at[len(copies)])

    add_copy("bre", bre_hbm, braw_ref.at[0])
    add_copy("bim", bim_hbm, braw_ref.at[1])
    for k in range(0, len(tiles), _DG):
        f0, f1 = tiles[k][0], min(F, tiles[k][0] + _DG * _FT)
        add_copy(("g", k), wg_hbm.at[f0:f1], wg_ref.at[f0:f1])
        add_copy(("u", k), wu_hbm.at[f0:f1], wu_ref.at[f0:f1])
    add_copy("cre", cre_hbm, ccat_ref.at[0])
    add_copy("cim", cim_hbm, ccat_ref.at[1])
    add_copy("wd", wd_hbm, wd_ref)

    @pl.when(step == 0)
    def _init():
        for c in copies.values():
            c.start()
        dt = jnp.exp(row(ldt_ref)).astype(bf16).astype(f32)
        lr = row(lre_ref)
        li = row(lim_ref)
        mag = jnp.exp(dt * lr)
        ar = mag * jnp.cos(dt * li)
        ai = mag * jnp.sin(dt * li)
        nr = ar - 1.0
        den = lr * lr + li * li
        cr = (nr * lr + ai * li) / den
        ci = (ai * lr - nr * li) / den
        rows = jax.lax.broadcasted_iota(jnp.int32, (8, P), 0)
        cct = jnp.where(rows == 0, cr, ci).T
        cr_c = cct[:, 0:1]
        ci_c = cct[:, 1:2]
        pw = [(ar, ai)]
        for _ in range(7):
            pr, pi = pw[-1]
            pw.append((pr * ar - pi * ai, pr * ai + pi * ar))
        for t, k in enumerate((1, 2, 4)):
            tab_ref[t, :, 0:P] = jnp.where(rows >= k, pw[k - 1][0], 0.0)
            tab_ref[t, :, P:2 * P] = jnp.where(rows >= k, pw[k - 1][1], 0.0)
        tab_ref[3, :, 0:P] = jnp.concatenate([p[0] for p in pw], axis=0)
        tab_ref[3, :, P:2 * P] = jnp.concatenate([p[1] for p in pw], axis=0)
        carry_ref[...] = jnp.zeros(carry_ref.shape, f32)
        copies["bre"].wait()
        copies["bim"].wait()
        bre = braw_ref[0].astype(f32)
        bim = braw_ref[1].astype(f32)
        bcat_ref[0:P, :] = (cr_c * bre - ci_c * bim).astype(bf16)
        bcat_ref[P:2 * P, :] = (cr_c * bim + ci_c * bre).astype(bf16)

    def body(first):
        def wait_first(*idx):
            if first:
                for i in idx:
                    copies[i].wait()

        x = x_ref[...]

        bu_ref[...] = jax.lax.dot_general(x, bcat_ref[...], _NT, preferred_element_type=f32)

        def scan_steps():
            c_re = carry_ref[0:1, 0:P]
            c_im = carry_ref[0:1, P:2 * P]
            for m in range(_T // 8):
                h_re = bu_ref[8 * m:8 * m + 8, 0:P]
                h_im = bu_ref[8 * m:8 * m + 8, P:2 * P]
                for t, k in enumerate((1, 2, 4)):
                    m_re = tab_ref[t, :, 0:P]
                    m_im = tab_ref[t, :, P:2 * P]
                    s_re = pltpu.roll(h_re, k, 0)
                    s_im = pltpu.roll(h_im, k, 0)
                    h_re, h_im = (h_re + (m_re * s_re - m_im * s_im),
                                  h_im + (m_re * s_im + m_im * s_re))
                p_re = tab_ref[3, :, 0:P]
                p_im = tab_ref[3, :, P:2 * P]
                h_re, h_im = (h_re + (p_re * c_re - p_im * c_im),
                              h_im + (p_re * c_im + p_im * c_re))
                c_re = h_re[7:8]
                c_im = h_im[7:8]
                if m % 2 == 0:
                    prev = (h_re, h_im)
                else:
                    r0 = 8 * (m - 1)
                    h_ref[r0:r0 + 16, 0:P] = jnp.concatenate(
                        [prev[0], h_re], axis=0).astype(bf16)
                    h_ref[r0:r0 + 16, P:2 * P] = jnp.concatenate(
                        [prev[1], h_im], axis=0).astype(bf16)
                yield
            carry_ref[0:1, 0:P] = c_re
            carry_ref[0:1, P:2 * P] = c_im
            yield

        scan = scan_steps()
        n_scan = _T // 8 + 1

        done = 0
        for k, (f0, fw) in enumerate(tiles):
            if k % _DG == 0:
                wait_first(("g", k), ("u", k))
                if k + _DG >= len(tiles):
                    wait_first("cre", "cim")
            gate = jax.lax.dot_general(x, wg_ref[f0:f0 + fw, :], _NT,
                                       preferred_element_type=f32)
            up = jax.lax.dot_general(x, wu_ref[f0:f0 + fw, :], _NT,
                                     preferred_element_type=f32)
            hid_ref[:, f0:f0 + fw] = (_gelu_tanh(gate) * up).astype(bf16)
            target = (n_scan * (k + 1)) // len(tiles)
            while done < target:
                next(scan)
                done += 1

        y = (jax.lax.dot_general(h_ref[:, 0:P], ccat_ref[0], _NT,
                                 preferred_element_type=f32)
             - jax.lax.dot_general(h_ref[:, P:2 * P], ccat_ref[1], _NT,
                                   preferred_element_type=f32))
        xf = x.astype(f32)
        a_out = 2.0 * y + xf * row(dskip_ref)

        wait_first("wd")
        b_out = jnp.dot(hid_ref[...], wd_ref[...], preferred_element_type=f32)

        s = jnp.sum(xf * row(gw_ref), axis=-1, keepdims=True)
        g = 1.0 / (1.0 + jnp.exp(-s))
        o_ref[...] = g * a_out + (1.0 - g) * b_out

    pl.when(step == 0)(lambda: body(True))
    pl.when(step != 0)(lambda: body(False))


@jax.jit
def pallas_gated_mix__ssm_conv_s5__geglu_ffn__prompt_kernel(
    A_x: jax.Array,
    A_Lambda_re: jax.Array,
    A_Lambda_im: jax.Array,
    A_B_re: jax.Array,
    A_B_im: jax.Array,
    A_C_re: jax.Array,
    A_C_im: jax.Array,
    A_log_dt: jax.Array,
    A_Dskip: jax.Array,
    B_x: jax.Array,
    B_w_gate: jax.Array,
    B_w_up: jax.Array,
    B_w_down: jax.Array,
    gate_w: jax.Array,
):
    Bsz, L, D = A_x.shape
    P = A_B_re.shape[0]
    F = B_w_gate.shape[1]
    assert Bsz == 1 and L % _T == 0
    x2 = A_x.reshape(L, D)

    full = lambda shape: pl.BlockSpec(shape, lambda i: (0,) * len(shape))
    hbm = pl.BlockSpec(memory_space=pl.ANY)

    out = pl.pallas_call(
        _kernel,
        grid=(L // _T,),
        in_specs=[
            pl.BlockSpec((_T, D), lambda i: (i, 0)),
            full((P,)), full((P,)), full((P,)),
            hbm, hbm,
            hbm, hbm,
            full((D,)),
            hbm, hbm, hbm,
            full((D,)),
        ],
        out_specs=pl.BlockSpec((_T, D), lambda i: (i, 0)),
        out_shape=jax.ShapeDtypeStruct((L, D), jnp.float32),
        scratch_shapes=[
            pltpu.VMEM((2, P, D), jnp.bfloat16),
            pltpu.VMEM((2 * P, D), jnp.bfloat16),
            pltpu.VMEM((2, D, P), jnp.bfloat16),
            pltpu.VMEM((4, 8, 2 * P), jnp.float32),
            pltpu.VMEM((8, 2 * P), jnp.float32),
            pltpu.VMEM((_T, 2 * P), jnp.bfloat16),
            pltpu.VMEM((_T, 2 * P), jnp.float32),
            pltpu.VMEM((_T, F), jnp.bfloat16),
            pltpu.VMEM((F, D), jnp.bfloat16),
            pltpu.VMEM((F, D), jnp.bfloat16),
            pltpu.VMEM((F, D), jnp.bfloat16),
            pltpu.SemaphoreType.DMA((5 + 2 * pl.cdiv(F, _DG * _FT),)),
        ],
        compiler_params=pltpu.CompilerParams(
            dimension_semantics=("arbitrary",),
            vmem_limit_bytes=100 * 1024 * 1024,
        ),
    )(x2, A_Lambda_re, A_Lambda_im, A_log_dt,
      A_B_re, A_B_im, A_C_re, A_C_im, A_Dskip,
      B_w_gate.T, B_w_up.T, B_w_down, gate_w)
    return out.reshape(Bsz, L, D)
```

```python
import jax
import jax.numpy as jnp
import jax.experimental.pallas as pl
import jax.experimental.pallas.tpu as pltpu

_T = 256
_FT = 128
_CW = 128
_DG = 4

_NT = (((1,), (1,)), ((), ()))


def _gelu_tanh(v):
    c = 0.7978845608028654
    return 0.5 * v * (1.0 + jnp.tanh(c * (v + 0.044715 * (v * v * v))))


def _kernel(x_ref, lre_ref, lim_ref, ldt_ref, bre_hbm, bim_hbm,
            cre_hbm, cim_hbm, dskip_ref, wg_hbm, wu_hbm, wd_hbm, gw_ref,
            o_ref,
            braw_ref, bcat_ref, ccat_ref, tab_ref, carry_ref, h_ref, bu_ref,
            hid_ref, wg_ref, wu_ref, wd_ref, sems):
    P = bre_hbm.shape[0]
    F = wd_ref.shape[0]
    step = pl.program_id(0)
    f32 = jnp.float32
    bf16 = jnp.bfloat16
    row = lambda r: r[...].astype(f32).reshape(1, r.shape[0])
    tiles = [(f0, min(_FT, F - f0)) for f0 in range(0, F, _FT)]

    copies = {}

    def add_copy(name, src, dst):
        copies[name] = pltpu.make_async_copy(src, dst, sems.at[len(copies)])

    add_copy("bre", bre_hbm, braw_ref.at[0])
    add_copy("bim", bim_hbm, braw_ref.at[1])
    for k in range(0, len(tiles), _DG):
        f0, f1 = tiles[k][0], min(F, tiles[k][0] + _DG * _FT)
        add_copy(("g", k), wg_hbm.at[f0:f1], wg_ref.at[f0:f1])
        add_copy(("u", k), wu_hbm.at[f0:f1], wu_ref.at[f0:f1])
    add_copy("cre", cre_hbm, ccat_ref.at[0])
    add_copy("cim", cim_hbm, ccat_ref.at[1])
    add_copy("wd", wd_hbm, wd_ref)

    @pl.when(step == 0)
    def _init():
        for c in copies.values():
            c.start()
        dt = jnp.exp(row(ldt_ref)).astype(bf16).astype(f32)
        lr = row(lre_ref)
        li = row(lim_ref)
        mag = jnp.exp(dt * lr)
        ar = mag * jnp.cos(dt * li)
        ai = mag * jnp.sin(dt * li)
        nr = ar - 1.0
        den = lr * lr + li * li
        cr = (nr * lr + ai * li) / den
        ci = (ai * lr - nr * li) / den
        rows = jax.lax.broadcasted_iota(jnp.int32, (8, P), 0)
        cct = jnp.where(rows == 0, cr, ci).T
        cr_c = cct[:, 0:1]
        ci_c = cct[:, 1:2]
        pw = [(ar, ai)]
        for _ in range(7):
            pr, pi = pw[-1]
            pw.append((pr * ar - pi * ai, pr * ai + pi * ar))
        for t, k in enumerate((1, 2, 4)):
            tab_ref[t, :, 0:P] = jnp.where(rows >= k, pw[k - 1][0], 0.0)
            tab_ref[t, :, P:2 * P] = jnp.where(rows >= k, pw[k - 1][1], 0.0)
        tab_ref[3, :, 0:P] = jnp.concatenate([p[0] for p in pw], axis=0)
        tab_ref[3, :, P:2 * P] = jnp.concatenate([p[1] for p in pw], axis=0)
        carry_ref[...] = jnp.zeros(carry_ref.shape, f32)
        copies["bre"].wait()
        copies["bim"].wait()
        bre = braw_ref[0].astype(f32)
        bim = braw_ref[1].astype(f32)
        bcat_ref[0:P, :] = (cr_c * bre - ci_c * bim).astype(bf16)
        bcat_ref[P:2 * P, :] = (cr_c * bim + ci_c * bre).astype(bf16)

    def body(first):
        def wait_first(*idx):
            if first:
                for i in idx:
                    copies[i].wait()

        x = x_ref[...]

        def ssm_group(c0, cw):
            re = slice(c0, c0 + cw)
            im = slice(P + c0, P + c0 + cw)
            bu_ref[:, re] = jax.lax.dot_general(x, bcat_ref[re, :], _NT,
                                                preferred_element_type=f32)
            bu_ref[:, im] = jax.lax.dot_general(x, bcat_ref[im, :], _NT,
                                                preferred_element_type=f32)
            c_re = carry_ref[0:1, re]
            c_im = carry_ref[0:1, im]
            for m in range(_T // 8):
                h_re = bu_ref[8 * m:8 * m + 8, re]
                h_im = bu_ref[8 * m:8 * m + 8, im]
                for t, k in enumerate((1, 2, 4)):
                    m_re = tab_ref[t, :, re]
                    m_im = tab_ref[t, :, im]
                    s_re = pltpu.roll(h_re, k, 0)
                    s_im = pltpu.roll(h_im, k, 0)
                    h_re, h_im = (h_re + (m_re * s_re - m_im * s_im),
                                  h_im + (m_re * s_im + m_im * s_re))
                p_re = tab_ref[3, :, re]
                p_im = tab_ref[3, :, im]
                h_re, h_im = (h_re + (p_re * c_re - p_im * c_im),
                              h_im + (p_re * c_im + p_im * c_re))
                c_re = h_re[7:8]
                c_im = h_im[7:8]
                if m % 2 == 0:
                    prev = (h_re, h_im)
                else:
                    r0 = 8 * (m - 1)
                    h_ref[r0:r0 + 16, re] = jnp.concatenate(
                        [prev[0], h_re], axis=0).astype(bf16)
                    h_ref[r0:r0 + 16, im] = jnp.concatenate(
                        [prev[1], h_im], axis=0).astype(bf16)
            carry_ref[0:1, re] = c_re
            carry_ref[0:1, im] = c_im

        ngrp = P // _CW
        at_tile = [[] for _ in tiles]
        for gi in range(ngrp):
            at_tile[min(len(tiles) - 1, 1 + (gi * (len(tiles) - 1)) // ngrp)].append(gi)

        for k, (f0, fw) in enumerate(tiles):
            if k % _DG == 0:
                wait_first(("g", k), ("u", k))
                if k + _DG >= len(tiles):
                    wait_first("cre", "cim")
            for gi in at_tile[k]:
                ssm_group(gi * _CW, _CW)
            gate = jax.lax.dot_general(x, wg_ref[f0:f0 + fw, :], _NT,
                                       preferred_element_type=f32)
            up = jax.lax.dot_general(x, wu_ref[f0:f0 + fw, :], _NT,
                                     preferred_element_type=f32)
            hid_ref[:, f0:f0 + fw] = (_gelu_tanh(gate) * up).astype(bf16)

        y = (jax.lax.dot_general(h_ref[:, 0:P], ccat_ref[0], _NT,
                                 preferred_element_type=f32)
             - jax.lax.dot_general(h_ref[:, P:2 * P], ccat_ref[1], _NT,
                                   preferred_element_type=f32))
        xf = x.astype(f32)
        a_out = 2.0 * y + xf * row(dskip_ref)

        wait_first("wd")
        b_out = jnp.dot(hid_ref[...], wd_ref[...], preferred_element_type=f32)

        s = jnp.sum(xf * row(gw_ref), axis=-1, keepdims=True)
        g = 1.0 / (1.0 + jnp.exp(-s))
        o_ref[...] = g * a_out + (1.0 - g) * b_out

    pl.when(step == 0)(lambda: body(True))
    pl.when(step != 0)(lambda: body(False))


@jax.jit
def pallas_gated_mix__ssm_conv_s5__geglu_ffn__prompt_kernel(
    A_x: jax.Array,
    A_Lambda_re: jax.Array,
    A_Lambda_im: jax.Array,
    A_B_re: jax.Array,
    A_B_im: jax.Array,
    A_C_re: jax.Array,
    A_C_im: jax.Array,
    A_log_dt: jax.Array,
    A_Dskip: jax.Array,
    B_x: jax.Array,
    B_w_gate: jax.Array,
    B_w_up: jax.Array,
    B_w_down: jax.Array,
    gate_w: jax.Array,
):
    Bsz, L, D = A_x.shape
    P = A_B_re.shape[0]
    F = B_w_gate.shape[1]
    assert Bsz == 1 and L % _T == 0 and P % _CW == 0
    x2 = A_x.reshape(L, D)

    full = lambda shape: pl.BlockSpec(shape, lambda i: (0,) * len(shape))
    hbm = pl.BlockSpec(memory_space=pl.ANY)

    out = pl.pallas_call(
        _kernel,
        grid=(L // _T,),
        in_specs=[
            pl.BlockSpec((_T, D), lambda i: (i, 0)),
            full((P,)), full((P,)), full((P,)),
            hbm, hbm,
            hbm, hbm,
            full((D,)),
            hbm, hbm, hbm,
            full((D,)),
        ],
        out_specs=pl.BlockSpec((_T, D), lambda i: (i, 0)),
        out_shape=jax.ShapeDtypeStruct((L, D), jnp.float32),
        scratch_shapes=[
            pltpu.VMEM((2, P, D), jnp.bfloat16),
            pltpu.VMEM((2 * P, D), jnp.bfloat16),
            pltpu.VMEM((2, D, P), jnp.bfloat16),
            pltpu.VMEM((4, 8, 2 * P), jnp.float32),
            pltpu.VMEM((8, 2 * P), jnp.float32),
            pltpu.VMEM((_T, 2 * P), jnp.bfloat16),
            pltpu.VMEM((_T, 2 * P), jnp.float32),
            pltpu.VMEM((_T, F), jnp.bfloat16),
            pltpu.VMEM((F, D), jnp.bfloat16),
            pltpu.VMEM((F, D), jnp.bfloat16),
            pltpu.VMEM((F, D), jnp.bfloat16),
            pltpu.SemaphoreType.DMA((5 + 2 * pl.cdiv(F, _DG * _FT),)),
        ],
        compiler_params=pltpu.CompilerParams(
            dimension_semantics=("arbitrary",),
            vmem_limit_bytes=100 * 1024 * 1024,
        ),
    )(x2, A_Lambda_re, A_Lambda_im, A_log_dt,
      A_B_re, A_B_im, A_C_re, A_C_im, A_Dskip,
      B_w_gate.T, B_w_up.T, B_w_down, gate_w)
    return out.reshape(Bsz, L, D)
```
